```python
import jax
import jax.numpy as jnp

def _softmax(x, axis=-1):
    return jax.nn.softmax(x, axis=axis)
def _gelu(x):
    return jax.nn.gelu(x, approximate=True)
def _silu(x):
    return jax.nn.silu(x)
def _sigmoid(x):
    return jax.nn.sigmoid(x)
def _layernorm(x, axis=-1, eps=1e-5):
    m = jnp.mean(x, axis=axis, keepdims=True)
    v = jnp.var(x, axis=axis, keepdims=True)
    return (x - m) / jnp.sqrt(v + eps)
def _scatter_add(tgt, idx, src, axis=0):
    return tgt.at[idx].add(src)
def _segment_sum(src, seg, n):
    return jax.ops.segment_sum(src, seg, n)
class _Rng:
    def __init__(self, key):
        self._k = key
    def _next(self):
        self._k, sub = jax.random.split(self._k)
        return sub
    def normal(self, shape):
        return jax.random.normal(self._next(), shape, dtype=jnp.bfloat16)
    def randint(self, lo, hi, shape):
        return jax.random.randint(self._next(), shape, lo, hi, dtype=jnp.int32)
    def uniform(self, shape, lo=0.0, hi=1.0):
        return jax.random.uniform(self._next(), shape, jnp.bfloat16, lo, hi)
    def permutation(self, n):
        return jax.random.permutation(self._next(), n)


kernel_name = 'standalone__structured_sparse_n_m__ragged'

def setup_inputs():
    _rng = _Rng(jax.random.key(int.from_bytes(__import__("os").urandom(4), "little")))
    _w = (lambda a: (lambda t: t.astype(jnp.bfloat16) if jnp.issubdtype(t.dtype, jnp.floating) else t)(jnp.asarray(a)))
    B, S, D = 16, 4096, 576
    assert D % 4 == 0, "d_model must be divisible by M=4 for 2:4 sparsity"
    return {
        "x": _w((lambda *s: _rng.normal(s) * 0.05)(B, S, D)),
        "w": _w((lambda *s: _rng.normal(s) * 0.05)(D, D)),
        "b": _w((lambda *s: _rng.normal(s) * 0.05)(D)),
    }

def reference(x, w, b):
    B, S, D = x.shape
    N, M = 2, 4
    G = D // M
    wg = w.reshape(G, M, D)
    mag = jnp.abs(wg)
    order = jnp.argsort(mag, 1)
    thr = jnp.take_along_axis(mag, order[:, M - N:M - N + 1, :], 1)
    mask = (lambda x, dt: x.astype(dt))(mag >= thr, w.dtype)
    wp = (wg * mask).reshape(D, D)
    return jnp.einsum("bsd,df->bsf", x, wp) + b
```

```python
import jax
import jax.numpy as jnp
from jax import lax
import jax.experimental.pallas as pl
import jax.experimental.pallas.tpu as pltpu

_FH = 288
_RING = 10
_IN_FIRST = (256, 256, 512, 1024, 2048)
_OUT_LAST = (2048, 1024, 512, 256, 256)


def _scheme():
    passes = {}

    def add(name, half, a, b):
        passes.setdefault(name, [None, None])[half] = (a, b)

    def strassen(k, l, p, q, s):
        t = 1 - s
        r = {"1": 1.0, "2": 2.0, "h": 0.5}[p]
        u0 = 2.0 if p == "h" else 1.0
        vs = (1.0, float(q))[s]
        h = k % 2
        add(f"I{s}", h, {(0, k): 1.0, (1, l): 1 / r}, {(k, t): 1.0, (l, s): -r})
        add(f"H1{q}", h, {(1, k): 1 / (r * vs), (1, l): 1 / (r * vs)}, {(k, t): 1.0})
        add(f"H0{q}", h, {(0, k): 1 / vs, (0, l): 1 / vs}, {(l, s): 1.0})
        add(f"G{s}{p}", h, {(0, k): 1 / u0}, {(k, s): 1.0, (l, s): -1.0})
        add(f"G{t}{p}", h, {(1, l): 1 / (r * u0)}, {(l, t): 1.0, (k, t): -1.0})
        add(f"O1{s}", h, {(1, k): 1 / r, (0, k): -1.0}, {(k, s): r, (k, t): -1.0})
        add(f"O0{t}", h, {(0, l): 1.0, (1, l): -1 / r}, {(l, t): 1.0, (l, s): -r})

    strassen(0, 2, "1", 1, 0)
    strassen(1, 3, "2", 2, 0)
    strassen(5, 7, "1", 1, 1)
    strassen(4, 6, "h", 2, 1)
    for j in range(2):
        add(f"G{j}2", 0, {(1, 8): 2 / 3, (0, 8): -1 / 3}, {(8, j): 1.0})
        add(f"G{j}h", 1, {(0, 8): 2 / 3, (1, 8): -1 / 3}, {(8, j): 1.0})
    return passes


_PASSES = _scheme()
_ORDER = ("G01", "G02", "G0h", "O00", "H11", "H12", "I0", "O10",
          "G11", "G12", "G1h", "O11", "H01", "H02", "I1", "O01")


def _prune_packed(u):
    mate = lax.broadcasted_iota(jnp.int32, u.shape, 0) ^ 1
    lo = pltpu.bitcast((u << 16) & 0x7FFFFFFF, jnp.float32)
    hi = pltpu.bitcast(u & 0x7FFF0000, jnp.float32)
    big, small = jnp.maximum(lo, hi), jnp.minimum(lo, hi)
    nbig = jnp.take_along_axis(big, mate, axis=0, mode="promise_in_bounds")
    nsmall = jnp.take_along_axis(small, mate, axis=0, mode="promise_in_bounds")
    thr = jnp.maximum(jnp.minimum(big, nbig), jnp.maximum(small, nsmall))
    return u & (jnp.where(lo < thr, 0, 0xFFFF) | jnp.where(hi < thr, 0, -65536))


def _prune_rows(w_bf16):
    u = pltpu.bitcast(w_bf16, jnp.int32)
    return [_prune_packed(u[8 * i:8 * i + 8]) for i in range(u.shape[0] // 8)]


def _combine(terms, block):
    acc = None
    for key, c in sorted(terms.items(), key=lambda e: -e[1]):
        v = block(key, abs(c))
        acc = v if acc is None else (acc + v if c > 0 else acc - v)
    return acc


def _super_tile(load, store, wa_ref, bias_ref):
    cache = {}

    def block(key, c):
        if (key, c) not in cache:
            cache[key, c] = load(*key).astype(jnp.float32) if c == 1 else block(key, 1.0) * c
        return cache[key, c]

    def mm(name):
        rhs = [load(*next(iter(b))) if len(b) == 1 else _combine(b, block).astype(jnp.bfloat16)
               for _, b in _PASSES[name]]
        return jnp.dot(pltpu.bitcast(wa_ref[_ORDER.index(name)], jnp.bfloat16),
                       jnp.concatenate(rhs, axis=0), preferred_element_type=jnp.float32)

    g1, g2, gh, o00 = mm("G01"), mm("G02"), mm("G0h"), mm("O00")
    s = g1 + g2 + gh
    c00 = s + gh + o00
    c10 = s + g2
    h1, h2, i0, o10 = mm("H11"), mm("H12"), mm("I0"), mm("O10")
    s = h1 + bias_ref[pl.ds(_FH, _FH)] + h2
    store(1, 0, c10 + s - i0 + o10)
    c11 = s + h2
    g1, g2, gh, o11 = mm("G11"), mm("G12"), mm("G1h"), mm("O11")
    s = g1 + g2 + gh
    c01 = i0 + (s + gh)
    c11 = c11 + (s + g2 + o11)
    h1, h2, i1, o01 = mm("H01"), mm("H02"), mm("I1"), mm("O01")
    s = h1 + bias_ref[pl.ds(0, _FH)] + h2
    store(0, 0, c00 + s + i1)
    store(0, 1, c01 + (s + h2) + o01)
    store(1, 1, c11 - i1)


def _split(sizes):
    return [(sum(sizes[:j]), sizes[j]) for j in range(len(sizes))]


def _kernel(x_hbm, w_hbm, b_hbm, o_hbm, xbuf, obuf, wbuf, bbuf, wa_ref, bias_ref,
            isem, fsem, osem, lsem, wsem):
    NB, D, S = x_hbm.shape
    NG = D // 64
    first, last = _split(_IN_FIRST), _split(_OUT_LAST)

    def x_first(j):
        o, n = first[j]
        return pltpu.make_async_copy(
            x_hbm.at[0, :, pl.ds(o, n)], xbuf.at[0, :, pl.ds(o, n)], fsem.at[j])

    def x_copy(t):
        return pltpu.make_async_copy(x_hbm.at[t], xbuf.at[t % _RING], isem.at[t % _RING])

    def o_start(b0, nb):
        for r0 in range(0, 64, 8):
            for t0 in range(0, S, 512):
                at = (pl.ds(r0, 8), pl.ds(t0, 512))
                pltpu.make_async_copy(
                    obuf.at[(pl.ds(b0 % _RING * NG, nb * NG), *at)],
                    o_hbm.at[(pl.ds(b0 * NG, nb * NG), *at)], osem.at[b0 // 2]).start()

    def o_wait(b0, nb):
        whole = obuf.at[pl.ds(b0 % _RING * NG, nb * NG)]
        pltpu.make_async_copy(whole, whole, osem.at[b0 // 2]).wait()

    def o_last(o, n):
        t = NB - 1
        return pltpu.make_async_copy(
            obuf.at[pl.ds(t % _RING * NG, NG), :, pl.ds(o, n)],
            o_hbm.at[pl.ds(t * NG, NG), :, pl.ds(o, n)], lsem)

    wrows = [(o, min(128, D - o)) for o in range(0, D, 128)]
    wcp = [pltpu.make_async_copy(w_hbm.at[pl.ds(o, n)], wbuf.at[pl.ds(o, n)], wsem.at[m])
           for m, (o, n) in enumerate(wrows)]
    bcp = pltpu.make_async_copy(b_hbm, bbuf, wsem.at[len(wrows)])
    bcp.start()
    for cp in wcp:
        cp.start()
    for j in range(len(first)):
        x_first(j).start()
    for t in range(1, _RING):
        x_copy(t).start()

    bcp.wait()
    bias_ref[...] = jnp.broadcast_to(bbuf[...].reshape(1, D).astype(jnp.float32), (128, D)).T
    tiles = []
    for m, (o, n) in enumerate(wrows):
        wcp[m].wait()
        parts = _prune_rows(wbuf[pl.ds(o, n), :]) * (128 // n)
        tiles.append(pltpu.bitcast(jnp.concatenate(parts, axis=0), jnp.bfloat16).T
                     .astype(jnp.float32))

    def w_block(key, c):
        v = tiles[key[1] // 2][key[0] * _FH:(key[0] + 1) * _FH]
        return v if c == 1 else v * c

    low = lax.broadcasted_iota(jnp.int32, (_FH, 128), 1) < 64
    for r, name in enumerate(_ORDER):
        (a0, _), (a1, _) = _PASSES[name]
        wa = jnp.where(low, _combine(a0, w_block), _combine(a1, w_block))
        wa_ref[r] = pltpu.bitcast(wa.astype(jnp.bfloat16), jnp.int32)

    def body(t, carry):
        u = t % _RING

        @pl.when(t > 0)
        def _():
            x_copy(t).wait()

        @pl.when((t > 0) & (t - 1 + _RING < NB))
        def _():
            x_copy(t - 1 + _RING).start()

        @pl.when((t >= _RING) & (t % 2 == 0))
        def _():
            o_wait(t - _RING, 2)

        for g0 in range(0, S, 256):
            for j, (o, n) in enumerate(first):
                if o == g0:
                    @pl.when(t == 0)
                    def _():
                        x_first(j).wait()

            if g0 == 0:
                @pl.when((t >= NB // 2) & (t < NB - 1))
                def _():
                    o_start(2 * t - NB, 2)

                @pl.when(t == NB - 1)
                def _():
                    o_start(NB - 2, 1)

            def load(k, j):
                return xbuf[u, pl.ds(64 * k, 64), pl.ds(g0 + 128 * j, 128)]

            def store(i, j, v):
                v = v.astype(obuf.dtype)
                r0 = i * _FH
                cuts = sorted({r0, r0 + _FH} | set(range(-(-r0 // 64) * 64, r0 + _FH, 64)))
                for lo, hi in zip(cuts[:-1], cuts[1:]):
                    obuf[u * NG + lo // 64, pl.ds(lo % 64, hi - lo), pl.ds(g0 + 128 * j, 128)] = (
                        v[lo - r0:hi - r0])

            _super_tile(load, store, wa_ref, bias_ref)

            for o, n in last:
                if o + n == g0 + 256:
                    @pl.when(t == NB - 1)
                    def _():
                        for oo in range(o, o + n, 256):
                            o_last(oo, 256).start()
        return carry

    lax.fori_loop(0, NB, body, 0)
    for b0 in range(NB - _RING, NB - 2, 2):
        o_wait(b0, 2)
    o_wait(NB - 2, 1)
    o_last(0, S).wait()


@jax.jit
def pallas_standalone__structured_sparse_n_m__ragged_kernel(
    x: jax.Array,
    w: jax.Array,
    b: jax.Array,
):
    B, S, D = x.shape
    xt = jnp.transpose(x, (0, 2, 1))
    out = pl.pallas_call(
        _kernel,
        in_specs=[pl.BlockSpec(memory_space=pl.ANY)] * 3,
        out_specs=pl.BlockSpec(memory_space=pl.ANY),
        out_shape=jax.ShapeDtypeStruct((B * D // 64, 64, S), x.dtype),
        scratch_shapes=[
            pltpu.VMEM((_RING, D, S), x.dtype),
            pltpu.VMEM((_RING * D // 64, 64, S), x.dtype),
            pltpu.VMEM((D, D), w.dtype),
            pltpu.VMEM((D,), b.dtype),
            pltpu.VMEM((len(_ORDER), _FH // 2, 128), jnp.int32),
            pltpu.VMEM((D, 128), jnp.float32),
            pltpu.SemaphoreType.DMA((_RING,)),
            pltpu.SemaphoreType.DMA((len(_IN_FIRST),)),
            pltpu.SemaphoreType.DMA((B // 2,)),
            pltpu.SemaphoreType.DMA(()),
            pltpu.SemaphoreType.DMA((6,)),
        ],
        compiler_params=pltpu.CompilerParams(
            vmem_limit_bytes=120 * 1024 * 1024,
            disable_bounds_checks=True,
            flags={"XLA_TPU_RESCHEDULE_DMA_DONES": True},
        ),
    )(xt, w, b)
    return jnp.transpose(out.reshape(B, D, S), (0, 2, 1))
```

```python
import jax
import jax.numpy as jnp
from jax import lax
import jax.experimental.pallas as pl
import jax.experimental.pallas.tpu as pltpu

_FH = 288
_RING = 5
_IN_FIRST = (256, 256, 512, 1024, 2048)
_OUT_LAST = (2048, 1024, 512, 256, 256)
_PASSES = ("H01", "H02", "H11", "H12", "G01", "G02", "G0h", "O10",
           "I0", "I1", "O00", "O01", "G11", "G12", "G1h", "O11")


def _prune_packed(u):
    mate = lax.broadcasted_iota(jnp.int32, u.shape, 0) ^ 1
    lo = pltpu.bitcast((u << 16) & 0x7FFFFFFF, jnp.float32)
    hi = pltpu.bitcast(u & 0x7FFF0000, jnp.float32)
    big, small = jnp.maximum(lo, hi), jnp.minimum(lo, hi)
    nbig = jnp.take_along_axis(big, mate, axis=0, mode="promise_in_bounds")
    nsmall = jnp.take_along_axis(small, mate, axis=0, mode="promise_in_bounds")
    thr = jnp.maximum(jnp.minimum(big, nbig), jnp.maximum(small, nsmall))
    return u & (jnp.where(lo < thr, 0, 0xFFFF) | jnp.where(hi < thr, 0, -65536))


def _prune_transposed(w):
    u = pltpu.bitcast(w, jnp.int32)
    parts = [_prune_packed(u[i:i + 8]) for i in range(0, u.shape[0], 8)]
    return pltpu.bitcast(jnp.concatenate(parts * (128 // w.shape[0]), axis=0), jnp.bfloat16).T


def _prepare_weights(tile, wa_ref):
    low = lax.broadcasted_iota(jnp.int32, (_FH // 2, 128), 1) < 64
    lane = lax.broadcasted_iota(jnp.int32, (_FH, 128), 1) < 64

    def rows(m):
        t = tile(m)
        return t[:_FH], t[_FH:]

    def f32(v, lo=1.0, hi=1.0):
        v = v.astype(jnp.float32)
        return v if lo == hi == 1.0 else v * jnp.where(lane, lo, hi)

    def put(name, lo, hi=None):
        lo = pltpu.bitcast(lo.astype(jnp.bfloat16), jnp.int32)
        if hi is not None:
            lo = jnp.where(low, lo, pltpu.bitcast(hi.astype(jnp.bfloat16), jnp.int32))
        wa_ref[_PASSES.index(name)] = lo

    a0, b0 = rows(0)
    b0s = f32(b0, 1.0, 0.5)
    put("O10", b0s - f32(a0))
    a1, b1 = rows(1)
    b1s = f32(b1, 1.0, 0.5)
    put("I0", f32(a0) + b1s)
    put("O01", f32(a1) - b1s)
    ha, hb = (f32(a0) + f32(a1)).astype(jnp.bfloat16), (b0s + b1s).astype(jnp.bfloat16)
    a2, b2 = rows(2)
    a2s = f32(a2, 0.5, 1.0)
    put("O11", f32(b2) - a2s)
    put("G11", b1, a2)
    a3, b3 = rows(3)
    a3s = f32(a3, 0.5, 1.0)
    put("I1", a2s + f32(b3))
    put("O00", a3s - f32(b3))
    put("G01", a0, b3)
    ha2, hb2 = (a2s + a3s).astype(jnp.bfloat16), (f32(b2) + f32(b3)).astype(jnp.bfloat16)
    put("H01", ha, ha2)
    put("H02", ha2, ha)
    put("H11", hb, hb2)
    put("H12", hb2, hb)
    a4, b4 = rows(4)
    tail = (f32(a4, -1 / 3, 2 / 3) + f32(b4, 2 / 3, -1 / 3)).astype(jnp.bfloat16)
    put("G02", tail, a0)
    put("G12", tail, b1s)
    put("G0h", b3, tail)
    put("G1h", a2s, tail)


def _super_tile(x, store, wa_ref, bias_ref):
    def diff(p, q, cp=1.0, cq=1.0):
        p, q = x(*p).astype(jnp.float32), x(*q).astype(jnp.float32)
        return ((p if cp == 1 else p * cp) - (q if cq == 1 else q * cq)).astype(jnp.bfloat16)

    def mm(name, lo, hi):
        return jnp.dot(pltpu.bitcast(wa_ref[_PASSES.index(name)], jnp.bfloat16),
                       jnp.concatenate([lo, hi], axis=0), preferred_element_type=jnp.float32)

    h01 = mm("H01", x(2, 0), x(7, 1))
    h02 = mm("H02", x(6, 1), x(3, 0))
    h11 = mm("H11", x(0, 1), x(5, 0))
    h12 = mm("H12", x(4, 0), x(1, 1))
    c00 = h01 + bias_ref[pl.ds(0, _FH)] + h02
    c01 = c00 + h02
    c10 = h11 + bias_ref[pl.ds(_FH, _FH)] + h12
    c11 = c10 + h12

    g1 = mm("G01", diff((0, 0), (2, 0)), diff((7, 0), (5, 0)))
    g2 = mm("G02", x(8, 0), diff((1, 0), (3, 0)))
    gh = mm("G0h", diff((6, 0), (4, 0)), x(8, 0))
    o10 = mm("O10", diff((0, 0), (0, 1)), diff((1, 0), (1, 1), cp=2.0))
    s = g1 + g2 + gh
    c00 = c00 + (s + gh)
    c10 = c10 + (s + g2) + o10

    i0 = mm("I0", diff((0, 1), (2, 0)), diff((1, 1), (3, 0), cq=2.0))
    i1 = mm("I1", diff((4, 0), (6, 1), cp=2.0), diff((5, 0), (7, 1)))
    o00 = mm("O00", diff((6, 0), (6, 1), cp=2.0), diff((7, 0), (7, 1)))
    o01 = mm("O01", diff((2, 1), (2, 0)), diff((3, 1), (3, 0), cq=2.0))
    store(1, 0, c10 - i0)
    store(0, 0, c00 + i1 + o00)
    c01 = c01 + i0 + o01
    c11 = c11 - i1

    g1 = mm("G11", diff((2, 1), (0, 1)), diff((5, 1), (7, 1)))
    g2 = mm("G12", x(8, 1), diff((3, 1), (1, 1)))
    gh = mm("G1h", diff((4, 1), (6, 1)), x(8, 1))
    o11 = mm("O11", diff((4, 1), (4, 0), cq=2.0), diff((5, 1), (5, 0)))
    s = g1 + g2 + gh
    store(0, 1, c01 + gh + s)
    store(1, 1, c11 + g2 + s + o11)


def _split(sizes):
    return [(sum(sizes[:j]), sizes[j]) for j in range(len(sizes))]


def _kernel(x_hbm, w_hbm, b_hbm, o_hbm, xbuf, obuf, wbuf, bbuf, wa_ref, bias_ref,
            isem, fsem, osem, wsem):
    NB, D, S = x_hbm.shape
    NP = NB // 2
    first = [(0, o, n) for o, n in _split(_IN_FIRST)] + [(1, 0, S)]

    def x_first(j):
        u, o, n = first[j]
        return pltpu.make_async_copy(
            x_hbm.at[u, :, pl.ds(o, n)], xbuf.at[u, :, pl.ds(o, n)], fsem.at[j])

    def x_pair(p):
        return pltpu.make_async_copy(
            x_hbm.at[pl.ds(2 * p, 2)], xbuf.at[pl.ds(p % _RING * 2, 2)], isem.at[p % _RING])

    def o_start(p, u, stride, rows, lo, hi):
        src, dst = (r.reshape(r.shape[0] * D // stride, stride, S) for r in (obuf, o_hbm))
        per_pair, n = 2 * D // stride, 8 * stride
        for r0 in rows:
            for c0 in range(lo, hi, n):
                at = (pl.ds(r0, 8), pl.ds(c0, n))
                pltpu.make_async_copy(
                    src.at[(pl.ds(p % _RING * per_pair + 9 * u, 9), *at)],
                    dst.at[(pl.ds(p * per_pair + 9 * u, 9), *at)], osem.at[p]).start()

    def o_wait(p):
        whole = obuf.at[pl.ds(p % _RING * 2, 2)]
        pltpu.make_async_copy(whole, whole, osem.at[p]).wait()

    wrows = [(o, min(128, D - o)) for o in range(0, D, 128)]
    wcp = [pltpu.make_async_copy(w_hbm.at[pl.ds(o, n)], wbuf.at[pl.ds(o, n)], wsem.at[m])
           for m, (o, n) in enumerate(wrows)]
    bcp = pltpu.make_async_copy(b_hbm, bbuf, wsem.at[len(wrows)])
    bcp.start()
    for cp in wcp:
        cp.start()
    for j in range(len(first)):
        x_first(j).start(priority=1)
    for p in range(1, _RING):
        x_pair(p).start(priority=1)

    def prepare():
        bcp.wait()
        bias_ref[...] = jnp.broadcast_to(bbuf[...].reshape(1, D).astype(jnp.float32), (128, D)).T

        def tile(m):
            wcp[m].wait()
            return _prune_transposed(wbuf[pl.ds(*wrows[m]), :])

        _prepare_weights(tile, wa_ref)

    def body(t, carry):
        pl.when(t == 0)(prepare)

        @pl.when(t > 0)
        def _():
            x_pair(t).wait()

        @pl.when((t > 0) & (t - 1 + _RING < NP))
        def _():
            x_pair(t - 1 + _RING).start(priority=1)

        @pl.when(t >= _RING)
        def _():
            o_wait(t - _RING)

        p = 2 * t - NP
        for u in range(2):
            slot = t % _RING * 2 + u
            for g in range(S // 256):
                g0 = 256 * g
                for j, (uu, o, n) in enumerate(first):
                    if (uu, o) == (u, g0):
                        @pl.when(t == 0)
                        def _():
                            x_first(j).wait()

                if (u, g) == (0, 0):
                    @pl.when((p == 0) | (t == NP - 1))
                    def _():
                        o_start(p, 0, 128, range(0, 128, 8), 0, S)
                if u == 1:
                    q = p + 1 + g // 8

                    @pl.when((p >= 0) & (q < NP - 1) & (q < t))
                    def _():
                        o_start(q, 0, 128, range(g % 8 * 16, g % 8 * 16 + 16, 8), 0, S)
                if u == 1 and g < 8 and g % 2 == 0:
                    @pl.when(t == NP - 1)
                    def _():
                        o_start(NP - 1, 0, 64, range(8 * g, 8 * g + 16, 8), 0, S)

                def load(k, j):
                    return xbuf[slot, pl.ds(64 * k, 64), pl.ds(g0 + 128 * j, 128)]

                def store(i, j, v):
                    obuf[slot, pl.ds(i * _FH, _FH), pl.ds(g0 + 128 * j, 128)] = v.astype(obuf.dtype)

                _super_tile(load, store, wa_ref, bias_ref)

                for o, n in _split(_OUT_LAST):
                    lag = (g0 + 256 - o - n) // 256
                    if u == 1 and n > 512 and 0 <= lag < n // 512:
                        @pl.when(t == NP - 1)
                        def _():
                            per = 64 * 512 // n
                            o_start(NP - 1, 1, 64, range(lag * per, lag * per + per, 8), o, o + n)
                    if u == 1 and n <= 512 and lag == 0:
                        @pl.when(t == NP - 1)
                        def _():
                            for c0 in range(o, o + n, 256):
                                pltpu.make_async_copy(
                                    obuf.at[(NP - 1) % _RING * 2 + 1, :, pl.ds(c0, 256)],
                                    o_hbm.at[NB - 1, :, pl.ds(c0, 256)], osem.at[NP - 1]).start()
        return carry

    lax.fori_loop(0, NP, body, 0)
    for p in range(NP - _RING, NP):
        o_wait(p)


@jax.jit
def pallas_standalone__structured_sparse_n_m__ragged_kernel(
    x: jax.Array,
    w: jax.Array,
    b: jax.Array,
):
    B, S, D = x.shape
    out = pl.pallas_call(
        _kernel,
        in_specs=[pl.BlockSpec(memory_space=pl.ANY)] * 3,
        out_specs=pl.BlockSpec(memory_space=pl.ANY),
        out_shape=jax.ShapeDtypeStruct((B, D, S), x.dtype),
        scratch_shapes=[
            pltpu.VMEM((2 * _RING, D, S), x.dtype),
            pltpu.VMEM((2 * _RING, D, S), x.dtype),
            pltpu.VMEM((D, D), w.dtype),
            pltpu.VMEM((D,), b.dtype),
            pltpu.VMEM((len(_PASSES), _FH // 2, 128), jnp.int32),
            pltpu.VMEM((D, 128), jnp.float32),
            pltpu.SemaphoreType.DMA((_RING,)),
            pltpu.SemaphoreType.DMA((len(_IN_FIRST) + 1,)),
            pltpu.SemaphoreType.DMA((B // 2,)),
            pltpu.SemaphoreType.DMA((6,)),
        ],
        compiler_params=pltpu.CompilerParams(
            vmem_limit_bytes=120 * 1024 * 1024,
            disable_bounds_checks=True,
            disable_semaphore_checks=True,
            flags={"XLA_TPU_RESCHEDULE_DMA_DONES": True},
        ),
    )(jnp.transpose(x, (0, 2, 1)), w, b)
    return jnp.transpose(out, (0, 2, 1))
```

```python
import jax
import jax.numpy as jnp
from jax import lax
import jax.experimental.pallas as pl
import jax.experimental.pallas.tpu as pltpu

_FH = 288
_RING = 5
_IN_FIRST = (256, 256, 512, 1024, 2048)
_OUT_LAST = (2048, 1024, 512, 256, 256)
_PASSES = ("H01", "H02", "H11", "H12", "G01", "G02", "G0h", "O10",
           "I0", "I1", "O00", "O01", "G11", "G12", "G1h", "O11")


def _prune_packed(u):
    mate = lax.broadcasted_iota(jnp.int32, u.shape, 0) ^ 1
    lo = pltpu.bitcast((u << 16) & 0x7FFFFFFF, jnp.float32)
    hi = pltpu.bitcast(u & 0x7FFF0000, jnp.float32)
    big, small = jnp.maximum(lo, hi), jnp.minimum(lo, hi)
    nbig = jnp.take_along_axis(big, mate, axis=0, mode="promise_in_bounds")
    nsmall = jnp.take_along_axis(small, mate, axis=0, mode="promise_in_bounds")
    thr = jnp.maximum(jnp.minimum(big, nbig), jnp.maximum(small, nsmall))
    return u & (jnp.where(lo < thr, 0, 0xFFFF) | jnp.where(hi < thr, 0, -65536))


def _prune_transposed(w):
    u = pltpu.bitcast(w, jnp.int32)
    parts = [_prune_packed(u[i:i + 8]) for i in range(0, u.shape[0], 8)]
    return pltpu.bitcast(jnp.concatenate(parts * (128 // w.shape[0]), axis=0), jnp.bfloat16).T


def _prepare_weights(tile, wa_ref):
    low = lax.broadcasted_iota(jnp.int32, (_FH // 2, 128), 1) < 64
    lane = lax.broadcasted_iota(jnp.int32, (_FH, 128), 1) < 64

    def rows(m):
        t = tile(m)
        return t[:_FH], t[_FH:]

    def f32(v, lo=1.0, hi=1.0):
        v = v.astype(jnp.float32)
        return v if lo == hi == 1.0 else v * jnp.where(lane, lo, hi)

    def put(name, lo, hi=None):
        lo = pltpu.bitcast(lo.astype(jnp.bfloat16), jnp.int32)
        if hi is not None:
            lo = jnp.where(low, lo, pltpu.bitcast(hi.astype(jnp.bfloat16), jnp.int32))
        wa_ref[_PASSES.index(name)] = lo

    a0, b0 = rows(0)
    b0s = f32(b0, 1.0, 0.5)
    put("O10", b0s - f32(a0))
    a1, b1 = rows(1)
    b1s = f32(b1, 1.0, 0.5)
    put("I0", f32(a0) + b1s)
    put("O01", f32(a1) - b1s)
    ha, hb = (f32(a0) + f32(a1)).astype(jnp.bfloat16), (b0s + b1s).astype(jnp.bfloat16)
    a2, b2 = rows(2)
    a2s = f32(a2, 0.5, 1.0)
    put("O11", f32(b2) - a2s)
    put("G11", b1, a2)
    a3, b3 = rows(3)
    a3s = f32(a3, 0.5, 1.0)
    put("I1", a2s + f32(b3))
    put("O00", a3s - f32(b3))
    put("G01", a0, b3)
    ha2, hb2 = (a2s + a3s).astype(jnp.bfloat16), (f32(b2) + f32(b3)).astype(jnp.bfloat16)
    put("H01", ha, ha2)
    put("H02", ha2, ha)
    put("H11", hb, hb2)
    put("H12", hb2, hb)
    a4, b4 = rows(4)
    tail = (f32(a4, -1 / 3, 2 / 3) + f32(b4, 2 / 3, -1 / 3)).astype(jnp.bfloat16)
    put("G02", tail, a0)
    put("G12", tail, b1s)
    put("G0h", b3, tail)
    put("G1h", a2s, tail)


def _super_tile(x, store, wa_ref, bias_ref, start_writes):
    def diff(p, q, cp=1.0, cq=1.0):
        p, q = x(*p).astype(jnp.float32), x(*q).astype(jnp.float32)
        return ((p if cp == 1 else p * cp) - (q if cq == 1 else q * cq)).astype(jnp.bfloat16)

    def mm(name, lo, hi):
        return jnp.dot(pltpu.bitcast(wa_ref[_PASSES.index(name)], jnp.bfloat16),
                       jnp.concatenate([lo, hi], axis=0), preferred_element_type=jnp.float32)

    start_writes("before")
    h01 = mm("H01", x(2, 0), x(7, 1))
    h02 = mm("H02", x(6, 1), x(3, 0))
    h11 = mm("H11", x(0, 1), x(5, 0))
    h12 = mm("H12", x(4, 0), x(1, 1))
    c00 = h01 + bias_ref[pl.ds(0, _FH)] + h02
    c01 = c00 + h02
    c10 = h11 + bias_ref[pl.ds(_FH, _FH)] + h12
    c11 = c10 + h12

    g1 = mm("G01", diff((0, 0), (2, 0)), diff((7, 0), (5, 0)))
    g2 = mm("G02", x(8, 0), diff((1, 0), (3, 0)))
    gh = mm("G0h", diff((6, 0), (4, 0)), x(8, 0))
    o10 = mm("O10", diff((0, 0), (0, 1)), diff((1, 0), (1, 1), cp=2.0))
    s = g1 + g2 + gh
    c00 = c00 + (s + gh)
    c10 = c10 + (s + g2) + o10

    i0 = mm("I0", diff((0, 1), (2, 0)), diff((1, 1), (3, 0), cq=2.0))
    i1 = mm("I1", diff((4, 0), (6, 1), cp=2.0), diff((5, 0), (7, 1)))
    o00 = mm("O00", diff((6, 0), (6, 1), cp=2.0), diff((7, 0), (7, 1)))
    o01 = mm("O01", diff((2, 1), (2, 0)), diff((3, 1), (3, 0), cq=2.0))
    store(1, 0, c10 - i0)
    store(0, 0, c00 + i1 + o00)
    start_writes("late")
    c01 = c01 + i0 + o01
    c11 = c11 - i1

    g1 = mm("G11", diff((2, 1), (0, 1)), diff((5, 1), (7, 1)))
    g2 = mm("G12", x(8, 1), diff((3, 1), (1, 1)))
    gh = mm("G1h", diff((4, 1), (6, 1)), x(8, 1))
    o11 = mm("O11", diff((4, 1), (4, 0), cq=2.0), diff((5, 1), (5, 0)))
    s = g1 + g2 + gh
    store(0, 1, c01 + gh + s)
    store(1, 1, c11 + g2 + s + o11)
    start_writes("after")


def _split(sizes):
    return [(sum(sizes[:j]), sizes[j]) for j in range(len(sizes))]


def _write_plan(NB, S):
    NP, G = NB // 2, S // 256

    def strided(groups, lo, hi):
        return [(groups(r), (r, 8), (c, 1024))
                for r in range(0, 128, 8) for c in range(lo, hi, 1024)]

    def pair(p):
        return strided(lambda r: (9 * p, 9), 0, S)

    bulk = [c for p in range(NP - 2) for c in pair(p)]
    plan = {(NP // 2 - 1, 2 * G - 1, "late"): bulk[:4], (NP // 2, 0, "before"): bulk[4:68]}
    done = 68
    for i in range((NP // 2 - 1) * G):
        t = NP // 2 + i // G
        end = min(76 + 8 * i, 64 * t)
        plan[t, G + i % G, "before"], done = bulk[done:end], end
    plan[NP - 1, 0, "before"] = pair(NP - 2)

    mid = 9 * (NP - 1) + 4
    part = strided(lambda r: (mid - 4, 5 if r < 64 else 4), 0, S)
    for i in range(len(part) // 16):
        plan[NP - 1, G + 2 * i, "before"] = part[16 * i:16 * i + 16]
    for o, n in _split(_OUT_LAST):
        if n >= 1024:
            part = strided(lambda r: (mid + 1, 4) if r < 64 else (mid, 5), o, o + n)
        else:
            part = [(g, r, (c, 256)) for c in range(o, o + n, 256)
                    for g, r in (((mid, 1), (64, 64)), ((mid + 1, 4), (0, 128)))]
        for i in range(0, len(part), 8):
            plan[NP - 1, G + (o + n) // 256 - 1 + i // 8, "after"] = part[i:i + 8]
    return plan


def _kernel(x_hbm, w_hbm, b_hbm, o_hbm, xbuf, obuf, wbuf, bbuf, wa_ref, bias_ref,
            isem, fsem, wsem, osem):
    NB, D, S = x_hbm.shape
    NP = NB // 2
    first = [(0, o, n) for o, n in _split(_IN_FIRST)] + [(1, 0, S)]
    plan = _write_plan(NB, S)

    def x_first(j):
        u, o, n = first[j]
        return pltpu.make_async_copy(
            x_hbm.at[u, :, pl.ds(o, n)], xbuf.at[u, :, pl.ds(o, n)], fsem.at[j])

    def x_pair(p):
        return pltpu.make_async_copy(
            x_hbm.at[pl.ds(2 * p, 2)], xbuf.at[pl.ds(p % _RING * 2, 2)], isem.at[p % _RING])

    def write(copies):
        for box in copies:
            at = tuple(pl.ds(o, n) for o, n in box)
            pltpu.make_async_copy(obuf.at[at], o_hbm.at[at], osem).start()

    wrows = [(o, min(128, D - o)) for o in range(0, D, 128)]
    wcp = [pltpu.make_async_copy(w_hbm.at[pl.ds(o, n)], wbuf.at[pl.ds(o, n)], wsem.at[m])
           for m, (o, n) in enumerate(wrows)]
    bcp = pltpu.make_async_copy(b_hbm, bbuf, wsem.at[len(wrows)])
    bcp.start()
    for cp in wcp:
        cp.start()
    for j in range(len(first)):
        x_first(j).start(priority=1)
    for p in range(1, _RING):
        x_pair(p).start(priority=1)

    def prepare():
        bcp.wait()
        bias_ref[...] = jnp.broadcast_to(bbuf[...].reshape(1, D).astype(jnp.float32), (128, D)).T

        def tile(m):
            wcp[m].wait()
            return _prune_transposed(wbuf[pl.ds(*wrows[m]), :])

        _prepare_weights(tile, wa_ref)

    def body(t, carry):
        pl.when(t == 0)(prepare)

        @pl.when(t > 0)
        def _():
            x_pair(t).wait()

        @pl.when((t > 0) & (t - 1 + _RING < NP))
        def _():
            x_pair(t - 1 + _RING).start(priority=1)

        for u in range(2):
            slot = t % _RING * 2 + u
            for g0 in range(0, S, 256):
                for j, (uu, o, n) in enumerate(first):
                    if (uu, o) == (u, g0):
                        pl.when(t == 0)(lambda: x_first(j).wait())

                def load(k, j):
                    return xbuf[slot, pl.ds(64 * k, 64), pl.ds(g0 + 128 * j, 128)]

                def store(i, j, v):
                    v = v.astype(obuf.dtype)
                    r0 = u * D + i * _FH
                    cuts = [r0, *range(r0 // 128 * 128 + 128, r0 + _FH, 128), r0 + _FH]
                    for lo, hi in zip(cuts[:-1], cuts[1:]):
                        obuf[9 * t + lo // 128, pl.ds(lo % 128, hi - lo),
                             pl.ds(g0 + 128 * j, 128)] = v[lo - r0:hi - r0]

                def start_writes(point):
                    for tt in range(NP):
                        copies = plan.get((tt, (u * S + g0) // 256, point))
                        if copies:
                            pl.when(t == tt)(lambda: write(copies))

                _super_tile(load, store, wa_ref, bias_ref, start_writes)
        return carry

    lax.fori_loop(0, NP, body, 0)
    pltpu.make_async_copy(obuf, obuf, osem).wait()


@jax.jit
def pallas_standalone__structured_sparse_n_m__ragged_kernel(
    x: jax.Array,
    w: jax.Array,
    b: jax.Array,
):
    B, S, D = x.shape
    out = pl.pallas_call(
        _kernel,
        in_specs=[pl.BlockSpec(memory_space=pl.ANY)] * 3,
        out_specs=pl.BlockSpec(memory_space=pl.ANY),
        out_shape=jax.ShapeDtypeStruct((B * D // 128, 128, S), x.dtype),
        scratch_shapes=[
            pltpu.VMEM((2 * _RING, D, S), x.dtype),
            pltpu.VMEM((B * D // 128, 128, S), x.dtype),
            pltpu.VMEM((D, D), w.dtype),
            pltpu.VMEM((D,), b.dtype),
            pltpu.VMEM((len(_PASSES), _FH // 2, 128), jnp.int32),
            pltpu.VMEM((D, 128), jnp.float32),
            pltpu.SemaphoreType.DMA((_RING,)),
            pltpu.SemaphoreType.DMA((len(_IN_FIRST) + 1,)),
            pltpu.SemaphoreType.DMA((6,)),
            pltpu.SemaphoreType.DMA(()),
        ],
        compiler_params=pltpu.CompilerParams(
            vmem_limit_bytes=124 * 1024 * 1024,
            disable_bounds_checks=True,
            disable_semaphore_checks=True,
            flags={"XLA_TPU_RESCHEDULE_DMA_DONES": True},
        ),
    )(jnp.transpose(x, (0, 2, 1)), w, b)
    return jnp.transpose(out.reshape(B, D, S), (0, 2, 1))
```

```python
import jax
import jax.numpy as jnp
from jax import lax
import jax.experimental.pallas as pl
import jax.experimental.pallas.tpu as pltpu

_FH = 288
_RING = 5
_IN_FIRST = (256, 256, 512, 1024, 2048)
_OUT_LAST = (2048, 1024, 512, 256, 256)
_PASSES = ("H01", "H02", "H11", "H12", "G01", "G02", "G0h", "O10",
           "I0", "I1", "O00", "O01", "G11", "G12", "G1h", "O11")


def _prune_packed(u):
    mate = lax.broadcasted_iota(jnp.int32, u.shape, 0) ^ 1
    lo = pltpu.bitcast((u << 16) & 0x7FFFFFFF, jnp.float32)
    hi = pltpu.bitcast(u & 0x7FFF0000, jnp.float32)
    big, small = jnp.maximum(lo, hi), jnp.minimum(lo, hi)
    nbig = jnp.take_along_axis(big, mate, axis=0, mode="promise_in_bounds")
    nsmall = jnp.take_along_axis(small, mate, axis=0, mode="promise_in_bounds")
    thr = jnp.maximum(jnp.minimum(big, nbig), jnp.maximum(small, nsmall))
    return u & (jnp.where(lo < thr, 0, 0xFFFF) | jnp.where(hi < thr, 0, -65536))


def _prune_transposed(w):
    u = pltpu.bitcast(w, jnp.int32)
    parts = [_prune_packed(u[i:i + 8]) for i in range(0, u.shape[0], 8)]
    return pltpu.bitcast(jnp.concatenate(parts * (128 // w.shape[0]), axis=0), jnp.bfloat16).T


def _prepare_weights(tile, wa_ref):
    low = lax.broadcasted_iota(jnp.int32, (_FH // 2, 128), 1) < 64
    lane = lax.broadcasted_iota(jnp.int32, (_FH, 128), 1) < 64

    def rows(m):
        t = tile(m)
        return t[:_FH], t[_FH:]

    def f32(v, lo=1.0, hi=1.0):
        v = v.astype(jnp.float32)
        return v if lo == hi == 1.0 else v * jnp.where(lane, lo, hi)

    def put(name, lo, hi=None):
        lo = pltpu.bitcast(lo.astype(jnp.bfloat16), jnp.int32)
        if hi is not None:
            lo = jnp.where(low, lo, pltpu.bitcast(hi.astype(jnp.bfloat16), jnp.int32))
        wa_ref[_PASSES.index(name)] = lo

    a0, b0 = rows(0)
    b0s = f32(b0, 1.0, 0.5)
    put("O10", b0s - f32(a0))
    a1, b1 = rows(1)
    b1s = f32(b1, 1.0, 0.5)
    put("I0", f32(a0) + b1s)
    put("O01", f32(a1) - b1s)
    ha, hb = (f32(a0) + f32(a1)).astype(jnp.bfloat16), (b0s + b1s).astype(jnp.bfloat16)
    a2, b2 = rows(2)
    a2s = f32(a2, 0.5, 1.0)
    put("O11", f32(b2) - a2s)
    put("G11", b1, a2)
    a3, b3 = rows(3)
    a3s = f32(a3, 0.5, 1.0)
    put("I1", a2s + f32(b3))
    put("O00", a3s - f32(b3))
    put("G01", a0, b3)
    ha2, hb2 = (a2s + a3s).astype(jnp.bfloat16), (f32(b2) + f32(b3)).astype(jnp.bfloat16)
    put("H01", ha, ha2)
    put("H02", ha2, ha)
    put("H11", hb, hb2)
    put("H12", hb2, hb)
    a4, b4 = rows(4)
    tail = (f32(a4, -1 / 3, 2 / 3) + f32(b4, 2 / 3, -1 / 3)).astype(jnp.bfloat16)
    put("G02", tail, a0)
    put("G12", tail, b1s)
    put("G0h", b3, tail)
    put("G1h", a2s, tail)


def _super_tile(x, store, wa_ref, bias_ref, start_writes):
    def diff(p, q, cp=1.0, cq=1.0):
        p, q = x(*p).astype(jnp.float32), x(*q).astype(jnp.float32)
        return ((p if cp == 1 else p * cp) - (q if cq == 1 else q * cq)).astype(jnp.bfloat16)

    def mm(name, lo, hi):
        return jnp.dot(pltpu.bitcast(wa_ref[_PASSES.index(name)], jnp.bfloat16),
                       jnp.concatenate([lo, hi], axis=0), preferred_element_type=jnp.float32)

    start_writes("before")
    h01 = mm("H01", x(2, 0), x(7, 1))
    h02 = mm("H02", x(6, 1), x(3, 0))
    h11 = mm("H11", x(0, 1), x(5, 0))
    h12 = mm("H12", x(4, 0), x(1, 1))
    c00 = h01 + bias_ref[pl.ds(0, _FH)] + h02
    c01 = c00 + h02
    c10 = h11 + bias_ref[pl.ds(_FH, _FH)] + h12
    c11 = c10 + h12

    g1 = mm("G01", diff((0, 0), (2, 0)), diff((7, 0), (5, 0)))
    g2 = mm("G02", x(8, 0), diff((1, 0), (3, 0)))
    gh = mm("G0h", diff((6, 0), (4, 0)), x(8, 0))
    o10 = mm("O10", diff((0, 0), (0, 1)), diff((1, 0), (1, 1), cp=2.0))
    s = g1 + g2 + gh
    c00 = c00 + (s + gh)
    c10 = c10 + (s + g2) + o10

    i0 = mm("I0", diff((0, 1), (2, 0)), diff((1, 1), (3, 0), cq=2.0))
    i1 = mm("I1", diff((4, 0), (6, 1), cp=2.0), diff((5, 0), (7, 1)))
    o00 = mm("O00", diff((6, 0), (6, 1), cp=2.0), diff((7, 0), (7, 1)))
    o01 = mm("O01", diff((2, 1), (2, 0)), diff((3, 1), (3, 0), cq=2.0))
    store(1, 0, c10 - i0)
    store(0, 0, c00 + i1 + o00)
    start_writes("late")
    c01 = c01 + i0 + o01
    c11 = c11 - i1

    g1 = mm("G11", diff((2, 1), (0, 1)), diff((5, 1), (7, 1)))
    g2 = mm("G12", x(8, 1), diff((3, 1), (1, 1)))
    gh = mm("G1h", diff((4, 1), (6, 1)), x(8, 1))
    o11 = mm("O11", diff((4, 1), (4, 0), cq=2.0), diff((5, 1), (5, 0)))
    s = g1 + g2 + gh
    store(0, 1, c01 + gh + s)
    store(1, 1, c11 + g2 + s + o11)
    start_writes("after")


def _split(sizes):
    return [(sum(sizes[:j]), sizes[j]) for j in range(len(sizes))]


def _write_plan(NB, S):
    NP, G = NB // 2, S // 256

    def strided(groups):
        return [(groups(r), (r, 8), (c, 1024)) for r in range(0, 128, 8) for c in range(0, S, 1024)]

    def pair(p):
        return strided(lambda r: (9 * p, 9))

    bulk = [c for p in range(NP - 2) for c in pair(p)]
    plan = {(NP // 2 - 1, 2 * G - 1, "late"): bulk[:4], (NP // 2, 0, "before"): bulk[4:68]}
    done = 68
    for i in range((NP // 2 - 1) * G):
        t = NP // 2 + i // G
        end = min(76 + 8 * i, 64 * t)
        plan[t, G + i % G, "before"], done = bulk[done:end], end
    plan[NP - 1, 0, "before"] = pair(NP - 2)

    mid = 9 * (NP - 1) + 4
    part = strided(lambda r: (mid - 4, 5 if r < 64 else 4))
    for i in range(len(part) // 16):
        plan[NP - 1, G + 2 * i, "before"] = part[16 * i:16 * i + 16]
    for o, n in _split(_OUT_LAST):
        if n >= 1024:
            part = [(g, (r + h, 8), (c, 1024))
                    for r in range(0, 64, 8) for c in range(o, o + n, 1024)
                    for g, h in (((mid + 1, 4), 0), ((mid, 5), 64))]
        else:
            part = [(g, r, (c, 256)) for c in range(o, o + n, 256)
                    for g, r in (((mid, 1), (64, 64)), ((mid + 1, 4), (0, 128)))]
        for i in range(0, len(part), 8):
            slot = (NP - 1, G + (o + n) // 256 - 1 + i // 8, "after")
            plan[slot] = plan.get(slot, []) + part[i:i + 8]
    assert sum(g[1] * r[1] * c[1] for cs in plan.values() for g, r, c in cs) == 9 * NP * 128 * S
    return plan


def _kernel(x_hbm, w_hbm, b_hbm, o_hbm, xbuf, obuf, wbuf, bbuf, wa_ref, bias_ref,
            isem, fsem, wsem, osem):
    NB, D, S = x_hbm.shape
    NP = NB // 2
    first = [(0, o, n) for o, n in _split(_IN_FIRST)] + [(1, 0, S)]
    plan = _write_plan(NB, S)

    def x_first(j):
        u, o, n = first[j]
        return pltpu.make_async_copy(
            x_hbm.at[u, :, pl.ds(o, n)], xbuf.at[u, :, pl.ds(o, n)], fsem.at[j])

    def x_pair(p):
        return pltpu.make_async_copy(
            x_hbm.at[pl.ds(2 * p, 2)], xbuf.at[pl.ds(p % _RING * 2, 2)], isem.at[p % _RING])

    def write(copies):
        for box in copies:
            at = tuple(pl.ds(o, n) for o, n in box)
            pltpu.make_async_copy(obuf.at[at], o_hbm.at[at], osem).start()

    wrows = [(o, min(128, D - o)) for o in range(0, D, 128)]
    wcp = [pltpu.make_async_copy(w_hbm.at[pl.ds(o, n)], wbuf.at[pl.ds(o, n)], wsem.at[m])
           for m, (o, n) in enumerate(wrows)]
    bcp = pltpu.make_async_copy(b_hbm, bbuf, wsem.at[len(wrows)])
    bcp.start()
    for cp in wcp:
        cp.start()
    for j in range(len(first)):
        x_first(j).start(priority=1)
    for p in range(1, _RING):
        x_pair(p).start(priority=1)

    def prepare():
        bcp.wait()
        bias_ref[...] = jnp.broadcast_to(bbuf[...].reshape(1, D).astype(jnp.float32), (128, D)).T

        def tile(m):
            wcp[m].wait()
            return _prune_transposed(wbuf[pl.ds(*wrows[m]), :])

        _prepare_weights(tile, wa_ref)

    def body(t, carry):
        pl.when(t == 0)(prepare)

        @pl.when(t > 0)
        def _():
            x_pair(t).wait()

        @pl.when((t > 0) & (t - 1 + _RING < NP))
        def _():
            x_pair(t - 1 + _RING).start(priority=1)

        for u in range(2):
            slot = t % _RING * 2 + u
            for g0 in range(0, S, 256):
                for j, (uu, o, n) in enumerate(first):
                    if (uu, o) == (u, g0):
                        pl.when(t == 0)(lambda: x_first(j).wait())

                def load(k, j):
                    return xbuf[slot, pl.ds(64 * k, 64), pl.ds(g0 + 128 * j, 128)]

                def store(i, j, v):
                    v = v.astype(obuf.dtype)
                    r0 = u * D + i * _FH
                    cuts = [r0, *range(r0 // 128 * 128 + 128, r0 + _FH, 128), r0 + _FH]
                    for lo, hi in zip(cuts[:-1], cuts[1:]):
                        obuf[9 * t + lo // 128, pl.ds(lo % 128, hi - lo),
                             pl.ds(g0 + 128 * j, 128)] = v[lo - r0:hi - r0]

                def start_writes(point):
                    for tt in range(NP):
                        copies = plan.get((tt, (u * S + g0) // 256, point))
                        if copies:
                            pl.when(t == tt)(lambda: write(copies))

                _super_tile(load, store, wa_ref, bias_ref, start_writes)
        return carry

    lax.fori_loop(0, NP, body, 0)
    pltpu.make_async_copy(obuf, obuf, osem).wait()


@jax.jit
def pallas_standalone__structured_sparse_n_m__ragged_kernel(
    x: jax.Array,
    w: jax.Array,
    b: jax.Array,
):
    B, S, D = x.shape
    out = pl.pallas_call(
        _kernel,
        in_specs=[pl.BlockSpec(memory_space=pl.ANY)] * 3,
        out_specs=pl.BlockSpec(memory_space=pl.ANY),
        out_shape=jax.ShapeDtypeStruct((B * D // 128, 128, S), x.dtype),
        scratch_shapes=[
            pltpu.VMEM((2 * _RING, D, S), x.dtype),
            pltpu.VMEM((B * D // 128, 128, S), x.dtype),
            pltpu.VMEM((D, D), w.dtype),
            pltpu.VMEM((D,), b.dtype),
            pltpu.VMEM((len(_PASSES), _FH // 2, 128), jnp.int32),
            pltpu.VMEM((D, 128), jnp.float32),
            pltpu.SemaphoreType.DMA((_RING,)),
            pltpu.SemaphoreType.DMA((len(_IN_FIRST) + 1,)),
            pltpu.SemaphoreType.DMA((6,)),
            pltpu.SemaphoreType.DMA(()),
        ],
        compiler_params=pltpu.CompilerParams(
            vmem_limit_bytes=124 * 1024 * 1024,
            disable_bounds_checks=True,
            disable_semaphore_checks=True,
            flags={"XLA_TPU_RESCHEDULE_DMA_DONES": True},
        ),
    )(jnp.transpose(x, (0, 2, 1)), w, b)
    return jnp.transpose(out.reshape(B, D, S), (0, 2, 1))
```

```python
import jax
import jax.numpy as jnp
from jax import lax
import jax.experimental.pallas as pl
import jax.experimental.pallas.tpu as pltpu

_FH = 288
_RING = 5
_IN_FIRST = (256, 256, 512, 1024, 2048)
_OUT_LAST = (2048, 1024, 512, 256, 256)
_PASSES = ("H01", "H02", "H11", "H12", "G01", "G02", "G0h", "O10",
           "I0", "I1", "O00", "O01", "G11", "G12", "G1h", "O11")


def _prune_packed(u):
    mate = lax.broadcasted_iota(jnp.int32, u.shape, 0) ^ 1
    lo = pltpu.bitcast((u << 16) & 0x7FFFFFFF, jnp.float32)
    hi = pltpu.bitcast(u & 0x7FFF0000, jnp.float32)
    big, small = jnp.maximum(lo, hi), jnp.minimum(lo, hi)
    nbig = jnp.take_along_axis(big, mate, axis=0, mode="promise_in_bounds")
    nsmall = jnp.take_along_axis(small, mate, axis=0, mode="promise_in_bounds")
    thr = jnp.maximum(jnp.minimum(big, nbig), jnp.maximum(small, nsmall))
    return u & (jnp.where(lo < thr, 0, 0xFFFF) | jnp.where(hi < thr, 0, -65536))


def _prune_transposed(w):
    u = pltpu.bitcast(w, jnp.int32)
    parts = [_prune_packed(u[i:i + 8]) for i in range(0, u.shape[0], 8)]
    return pltpu.bitcast(jnp.concatenate(parts * (128 // w.shape[0]), axis=0), jnp.bfloat16).T


def _prepare_weights(tile, wa_ref, down_ref):
    low = lax.broadcasted_iota(jnp.int32, (_FH // 2, 128), 1) < 64
    lane = lax.broadcasted_iota(jnp.int32, (1, 128), 1) < 64

    def put(name, lo, hi=None):
        lo = pltpu.bitcast(lo.astype(jnp.bfloat16), jnp.int32)
        if hi is not None:
            lo = jnp.where(low, lo, pltpu.bitcast(hi.astype(jnp.bfloat16), jnp.int32))
        wa_ref[_PASSES.index(name)] = lo

    def pow2(e):
        return pltpu.bitcast((127 + e) << 23, jnp.float32)

    def balanced(m, half_a, half_b):
        tiles = [tile(m).astype(jnp.float32), tile(m + 1).astype(jnp.float32)]
        exps = [pltpu.bitcast(jnp.max(jnp.abs(t), axis=0, keepdims=True), jnp.int32) >> 23
                for t in tiles]
        out = []
        for i, (t, e) in enumerate(zip(tiles, exps)):
            d = jnp.minimum(jnp.maximum(exps[0], exps[1]) - e, 126)
            down_ref[pl.ds(128 * (m + i), 128)] = jnp.broadcast_to(pow2(-d), (128, 128)).T
            out += [t[:_FH] * (pow2(d) * half_a), t[_FH:] * (pow2(d) * half_b), pow2(-d)]
        return out

    a0, b0, down0, a1, b1, down1 = balanced(0, 1.0, jnp.where(lane, 1.0, 0.5))
    put("O10", b0 - a0)
    put("I0", a0 + b1)
    put("O01", a1 - b1)
    ha, hb = ((a0 + a1) * down1).astype(jnp.bfloat16), ((b0 + b1) * down0).astype(jnp.bfloat16)
    a0, b1 = a0.astype(jnp.bfloat16), b1.astype(jnp.bfloat16)
    a2, b2, down2, a3, b3, down3 = balanced(2, jnp.where(lane, 0.5, 1.0), 1.0)
    put("O11", b2 - a2)
    put("I1", a2 + b3)
    put("O00", a3 - b3)
    ha2, hb2 = ((a2 + a3) * down3).astype(jnp.bfloat16), ((b2 + b3) * down2).astype(jnp.bfloat16)
    a2, b3 = a2.astype(jnp.bfloat16), b3.astype(jnp.bfloat16)
    put("G11", b1, a2)
    put("G01", a0, b3)
    put("H01", ha, ha2)
    put("H02", ha2, ha)
    put("H11", hb, hb2)
    put("H12", hb2, hb)
    t = tile(4).astype(jnp.float32)
    tail = (t[:_FH] * jnp.where(lane, -1 / 3, 2 / 3)
            + t[_FH:] * jnp.where(lane, 2 / 3, -1 / 3)).astype(jnp.bfloat16)
    put("G02", tail, a0)
    put("G12", tail, b1)
    put("G0h", b3, tail)
    put("G1h", a2, tail)


def _super_tile(x, store, wa_ref, down_ref, bias_ref, start_writes):
    def diff(p, q, cp=1.0, cq=1.0):
        p, q = (x(k, j).astype(jnp.float32) * down_ref[pl.ds(64 * k, 64)] for k, j in (p, q))
        return ((p if cp == 1 else p * cp) - (q if cq == 1 else q * cq)).astype(jnp.bfloat16)

    def mm(name, lo, hi):
        return jnp.dot(pltpu.bitcast(wa_ref[_PASSES.index(name)], jnp.bfloat16),
                       jnp.concatenate([lo, hi], axis=0), preferred_element_type=jnp.float32)

    start_writes("before")
    h01 = mm("H01", x(2, 0), x(7, 1))
    h02 = mm("H02", x(6, 1), x(3, 0))
    h11 = mm("H11", x(0, 1), x(5, 0))
    h12 = mm("H12", x(4, 0), x(1, 1))
    c00 = h01 + bias_ref[pl.ds(0, _FH)] + h02
    c01 = c00 + h02
    c10 = h11 + bias_ref[pl.ds(_FH, _FH)] + h12
    c11 = c10 + h12

    g1 = mm("G01", diff((0, 0), (2, 0)), diff((7, 0), (5, 0)))
    g2 = mm("G02", x(8, 0), diff((1, 0), (3, 0)))
    gh = mm("G0h", diff((6, 0), (4, 0)), x(8, 0))
    o10 = mm("O10", diff((0, 0), (0, 1)), diff((1, 0), (1, 1), cp=2.0))
    s = g1 + g2 + gh
    c00 = c00 + (s + gh)
    c10 = c10 + (s + g2) + o10

    i0 = mm("I0", diff((0, 1), (2, 0)), diff((1, 1), (3, 0), cq=2.0))
    i1 = mm("I1", diff((4, 0), (6, 1), cp=2.0), diff((5, 0), (7, 1)))
    o00 = mm("O00", diff((6, 0), (6, 1), cp=2.0), diff((7, 0), (7, 1)))
    o01 = mm("O01", diff((2, 1), (2, 0)), diff((3, 1), (3, 0), cq=2.0))
    store(1, 0, c10 - i0)
    store(0, 0, c00 + i1 + o00)
    start_writes("late")
    c01 = c01 + i0 + o01
    c11 = c11 - i1

    g1 = mm("G11", diff((2, 1), (0, 1)), diff((5, 1), (7, 1)))
    g2 = mm("G12", x(8, 1), diff((3, 1), (1, 1)))
    gh = mm("G1h", diff((4, 1), (6, 1)), x(8, 1))
    o11 = mm("O11", diff((4, 1), (4, 0), cq=2.0), diff((5, 1), (5, 0)))
    s = g1 + g2 + gh
    store(0, 1, c01 + gh + s)
    store(1, 1, c11 + g2 + s + o11)
    start_writes("after")


def _split(sizes):
    return [(sum(sizes[:j]), sizes[j]) for j in range(len(sizes))]


def _write_plan(NB, S):
    NP, G = NB // 2, S // 256

    def strided(groups):
        return [(groups(r), (r, 8), (c, 1024)) for r in range(0, 128, 8) for c in range(0, S, 1024)]

    def pair(p):
        return strided(lambda r: (9 * p, 9))

    bulk = [c for p in range(NP - 2) for c in pair(p)]
    plan = {(NP // 2 - 1, 2 * G - 1, "late"): bulk[:4], (NP // 2, 0, "before"): bulk[4:68]}
    done = 68
    for i in range((NP // 2 - 1) * G):
        t = NP // 2 + i // G
        end = min(76 + 8 * i, 64 * t)
        plan[t, G + i % G, "before"], done = bulk[done:end], end
    plan[NP - 1, 0, "before"] = pair(NP - 2)

    mid = 9 * (NP - 1) + 4
    part = strided(lambda r: (mid - 4, 5 if r < 64 else 4))
    for i in range(len(part) // 16):
        plan[NP - 1, G + 2 * i, "before"] = part[16 * i:16 * i + 16]
    for o, n in _split(_OUT_LAST):
        if n >= 1024:
            part = [(g, (r + h, 8), (c, 1024))
                    for r in range(0, 64, 8) for c in range(o, o + n, 1024)
                    for g, h in (((mid + 1, 4), 0), ((mid, 5), 64))]
        else:
            part = [(g, r, (c, 256)) for c in range(o, o + n, 256)
                    for g, r in (((mid, 1), (64, 64)), ((mid + 1, 4), (0, 128)))]
        for i in range(0, len(part), 8):
            slot = (NP - 1, G + (o + n) // 256 - 1 + i // 8, "after")
            plan[slot] = plan.get(slot, []) + part[i:i + 8]
    assert sum(g[1] * r[1] * c[1] for cs in plan.values() for g, r, c in cs) == 9 * NP * 128 * S
    return plan


def _kernel(x_hbm, w_hbm, b_hbm, o_hbm, xbuf, obuf, wbuf, bbuf, wa_ref, down_ref, bias_ref,
            isem, fsem, wsem, osem):
    NB, D, S = x_hbm.shape
    NP = NB // 2
    first = [(0, o, n) for o, n in _split(_IN_FIRST)] + [(1, 0, S)]
    plan = _write_plan(NB, S)

    def x_first(j):
        u, o, n = first[j]
        return pltpu.make_async_copy(
            x_hbm.at[u, :, pl.ds(o, n)], xbuf.at[u, :, pl.ds(o, n)], fsem.at[j])

    def x_pair(p):
        return pltpu.make_async_copy(
            x_hbm.at[pl.ds(2 * p, 2)], xbuf.at[pl.ds(p % _RING * 2, 2)], isem.at[p % _RING])

    def write(copies):
        for box in copies:
            at = tuple(pl.ds(o, n) for o, n in box)
            pltpu.make_async_copy(obuf.at[at], o_hbm.at[at], osem).start()

    wrows = [(o, min(128, D - o)) for o in range(0, D, 128)]
    wcp = [pltpu.make_async_copy(w_hbm.at[pl.ds(o, n)], wbuf.at[pl.ds(o, n)], wsem.at[m])
           for m, (o, n) in enumerate(wrows)]
    bcp = pltpu.make_async_copy(b_hbm, bbuf, wsem.at[len(wrows)])
    bcp.start()
    for cp in wcp:
        cp.start()
    for j in range(len(first)):
        x_first(j).start(priority=1)
    for p in range(1, _RING):
        x_pair(p).start(priority=1)

    def prepare():
        bcp.wait()
        bias_ref[...] = jnp.broadcast_to(bbuf[...].reshape(1, D).astype(jnp.float32), (128, D)).T

        def tile(m):
            wcp[m].wait()
            return _prune_transposed(wbuf[pl.ds(*wrows[m]), :])

        _prepare_weights(tile, wa_ref, down_ref)

    def body(t, carry):
        pl.when(t == 0)(prepare)

        @pl.when(t > 0)
        def _():
            x_pair(t).wait()

        @pl.when((t > 0) & (t - 1 + _RING < NP))
        def _():
            x_pair(t - 1 + _RING).start(priority=1)

        for u in range(2):
            slot = t % _RING * 2 + u
            for g0 in range(0, S, 256):
                for j, (uu, o, n) in enumerate(first):
                    if (uu, o) == (u, g0):
                        pl.when(t == 0)(lambda: x_first(j).wait())

                def load(k, j):
                    return xbuf[slot, pl.ds(64 * k, 64), pl.ds(g0 + 128 * j, 128)]

                def store(i, j, v):
                    v = v.astype(obuf.dtype)
                    r0 = u * D + i * _FH
                    cuts = [r0, *range(r0 // 128 * 128 + 128, r0 + _FH, 128), r0 + _FH]
                    for lo, hi in zip(cuts[:-1], cuts[1:]):
                        obuf[9 * t + lo // 128, pl.ds(lo % 128, hi - lo),
                             pl.ds(g0 + 128 * j, 128)] = v[lo - r0:hi - r0]

                def start_writes(point):
                    for tt in range(NP):
                        copies = plan.get((tt, (u * S + g0) // 256, point))
                        if copies:
                            pl.when(t == tt)(lambda: write(copies))

                _super_tile(load, store, wa_ref, down_ref, bias_ref, start_writes)
        return carry

    lax.fori_loop(0, NP, body, 0)
    pltpu.make_async_copy(obuf, obuf, osem).wait()


@jax.jit
def pallas_standalone__structured_sparse_n_m__ragged_kernel(
    x: jax.Array,
    w: jax.Array,
    b: jax.Array,
):
    B, S, D = x.shape
    out = pl.pallas_call(
        _kernel,
        in_specs=[pl.BlockSpec(memory_space=pl.ANY)] * 3,
        out_specs=pl.BlockSpec(memory_space=pl.ANY),
        out_shape=jax.ShapeDtypeStruct((B * D // 128, 128, S), x.dtype),
        scratch_shapes=[
            pltpu.VMEM((2 * _RING, D, S), x.dtype),
            pltpu.VMEM((B * D // 128, 128, S), x.dtype),
            pltpu.VMEM((D, D), w.dtype),
            pltpu.VMEM((D,), b.dtype),
            pltpu.VMEM((len(_PASSES), _FH // 2, 128), jnp.int32),
            pltpu.VMEM((512, 128), jnp.float32),
            pltpu.VMEM((D, 128), jnp.float32),
            pltpu.SemaphoreType.DMA((_RING,)),
            pltpu.SemaphoreType.DMA((len(_IN_FIRST) + 1,)),
            pltpu.SemaphoreType.DMA((6,)),
            pltpu.SemaphoreType.DMA(()),
        ],
        compiler_params=pltpu.CompilerParams(
            vmem_limit_bytes=124 * 1024 * 1024,
            disable_bounds_checks=True,
            disable_semaphore_checks=True,
            flags={"XLA_TPU_RESCHEDULE_DMA_DONES": True},
        ),
    )(jnp.transpose(x, (0, 2, 1)), w, b)
    return jnp.transpose(out.reshape(B, D, S), (0, 2, 1))
```

```python
import functools

import jax
import jax.numpy as jnp
from jax import lax
import jax.experimental.pallas as pl
import jax.experimental.pallas.tpu as pltpu

_FH = 288
_RING = 5
_IN_FIRST = (256, 256, 512, 1024, 2048)
_OUT_LAST = (2048, 1024, 512, 256, 256)
_SAFE = 0.75
_PASSES = ("H01", "H02", "H11", "H12", "G01", "G02", "G0h", "O10",
           "I0", "I1", "O00", "O01", "G11", "G12", "G1h", "O11")


def _prune_packed(u):
    mate = lax.broadcasted_iota(jnp.int32, u.shape, 0) ^ 1
    lo = pltpu.bitcast((u << 16) & 0x7FFFFFFF, jnp.float32)
    hi = pltpu.bitcast(u & 0x7FFF0000, jnp.float32)
    big, small = jnp.maximum(lo, hi), jnp.minimum(lo, hi)
    nbig = jnp.take_along_axis(big, mate, axis=0, mode="promise_in_bounds")
    nsmall = jnp.take_along_axis(small, mate, axis=0, mode="promise_in_bounds")
    thr = jnp.maximum(jnp.minimum(big, nbig), jnp.maximum(small, nsmall))
    return u & (jnp.where(lo < thr, 0, 0xFFFF) | jnp.where(hi < thr, 0, -65536))


def _prune(w):
    u = pltpu.bitcast(w, jnp.int32)
    parts = [_prune_packed(u[i:i + 8]) for i in range(0, u.shape[0], 8)]
    return pltpu.bitcast(jnp.concatenate(parts, axis=0), jnp.bfloat16)


def _prepare_weights(tile, wa_ref):
    low = lax.broadcasted_iota(jnp.int32, (_FH, 128), 1) < 64

    def rows(m):
        t = tile(m).astype(jnp.float32)
        return t[:_FH], t[_FH:]

    def put(name, lo, hi=None):
        v = lo if hi is None else jnp.where(low, lo, hi)
        wa_ref[_PASSES.index(name)] = v.astype(wa_ref.dtype)

    a0, b0 = rows(0)
    b0 = b0 * jnp.where(low, 1.0, 0.5)
    put("O10", b0 - a0)
    a1, b1 = rows(1)
    b1 = b1 * jnp.where(low, 1.0, 0.5)
    put("I0", a0 + b1)
    put("O01", a1 - b1)
    ha, hb = a0 + a1, b0 + b1
    a2, b2 = rows(2)
    a2 = a2 * jnp.where(low, 0.5, 1.0)
    put("O11", b2 - a2)
    put("G11", b1, a2)
    a3, b3 = rows(3)
    a3 = a3 * jnp.where(low, 0.5, 1.0)
    put("I1", a2 + b3)
    put("O00", a3 - b3)
    put("G01", a0, b3)
    ha2, hb2 = a2 + a3, b2 + b3
    put("H01", ha, ha2)
    put("H02", ha2, ha)
    put("H11", hb, hb2)
    put("H12", hb2, hb)
    a4, b4 = rows(4)
    tail = a4 * jnp.where(low, -1 / 3, 2 / 3) + b4 * jnp.where(low, 2 / 3, -1 / 3)
    put("G02", tail, a0)
    put("G12", tail, b1)
    put("G0h", b3, tail)
    put("G1h", a2, tail)


def _fold(op, v):
    return functools.reduce(op, [v[i:i + 8] for i in range(0, v.shape[0], 8)])


def _quartic(v):
    v = v.astype(jnp.float32)
    v = v * v
    return _fold(jnp.add, v * v)


def _super_tile(x, store, wa_ref, bias_ref, start_writes):
    quartic = {}

    def wide(k, j):
        v = x(k, j).astype(jnp.float32)
        if (k, j) not in quartic:
            quartic[k, j] = _quartic(v)
        return v

    def diff(p, q, cp=1.0, cq=1.0):
        p, q = wide(*p), wide(*q)
        return (p if cp == 1 else p * cp) - (q if cq == 1 else q * cq)

    def mm(name, lo, hi):
        rhs = jnp.concatenate([lo, hi], axis=0).astype(jnp.bfloat16)
        return jnp.dot(wa_ref[_PASSES.index(name)], rhs, preferred_element_type=jnp.float32)

    start_writes("before")
    h01 = mm("H01", x(2, 0), x(7, 1))
    h02 = mm("H02", x(6, 1), x(3, 0))
    h11 = mm("H11", x(0, 1), x(5, 0))
    h12 = mm("H12", x(4, 0), x(1, 1))
    c00 = h01 + bias_ref[pl.ds(0, _FH)] + h02
    c01 = c00 + h02
    c10 = h11 + bias_ref[pl.ds(_FH, _FH)] + h12
    c11 = c10 + h12

    g1 = mm("G01", diff((0, 0), (2, 0)), diff((7, 0), (5, 0)))
    g2 = mm("G02", wide(8, 0), diff((1, 0), (3, 0)))
    gh = mm("G0h", diff((6, 0), (4, 0)), wide(8, 0))
    o10 = mm("O10", diff((0, 0), (0, 1)), diff((1, 0), (1, 1), cp=2.0))
    s = g1 + g2 + gh
    c00 = c00 + (s + gh)
    c10 = c10 + (s + g2) + o10

    i0 = mm("I0", diff((0, 1), (2, 0)), diff((1, 1), (3, 0), cq=2.0))
    i1 = mm("I1", diff((4, 0), (6, 1), cp=2.0), diff((5, 0), (7, 1)))
    o00 = mm("O00", diff((6, 0), (6, 1), cp=2.0), diff((7, 0), (7, 1)))
    o01 = mm("O01", diff((2, 1), (2, 0)), diff((3, 1), (3, 0), cq=2.0))
    store(1, 0, c10 - i0)
    store(0, 0, c00 + i1 + o00)
    c01 = c01 + i0 + o01
    c11 = c11 - i1

    g1 = mm("G11", diff((2, 1), (0, 1)), diff((5, 1), (7, 1)))
    g2 = mm("G12", wide(8, 1), diff((3, 1), (1, 1)))
    gh = mm("G1h", diff((4, 1), (6, 1)), wide(8, 1))
    o11 = mm("O11", diff((4, 1), (4, 0), cq=2.0), diff((5, 1), (5, 0)))
    s = g1 + g2 + gh
    store(0, 1, c01 + gh + s)
    store(1, 1, c11 + g2 + s + o11)
    start_writes("after")
    return jnp.maximum(*(
        jnp.sum(functools.reduce(jnp.add, [quartic[k, j] for k in range(9)]), axis=0, keepdims=True)
        for j in range(2)))


def _split(sizes):
    return [(sum(sizes[:j]), sizes[j]) for j in range(len(sizes))]


def _write_plan(NB, S):
    NP, G = NB // 2, S // 256

    def strided(groups):
        return [(groups(r), (r, 8), (c, 1024)) for r in range(0, 128, 8) for c in range(0, S, 1024)]

    def pair(p):
        return strided(lambda r: (9 * p, 9))

    bulk = [c for p in range(NP - 2) for c in pair(p)]
    plan = {(NP // 2 - 1, 2 * G - 1, "late"): bulk[:16], (NP // 2, 0, "before"): bulk[16:68]}
    done = 68
    for i in range((NP // 2 - 1) * G):
        t = NP // 2 + i // G
        end = min(76 + 8 * i, 64 * t)
        plan[t, G + i % G, "before"], done = bulk[done:end], end
    plan[NP - 1, 0, "before"] = pair(NP - 2)

    mid = 9 * (NP - 1) + 4
    part = strided(lambda r: (mid - 4, 5 if r < 64 else 4))
    for i in range(len(part) // 16):
        plan[NP - 1, G + 2 * i, "before"] = part[16 * i:16 * i + 16]
    for o, n in _split(_OUT_LAST):
        if n >= 1024:
            part = [(g, (r + h, 8), (c, 1024))
                    for r in range(0, 64, 8) for c in range(o, o + n, 1024)
                    for g, h in (((mid + 1, 4), 0), ((mid, 5), 64))]
        else:
            part = [(g, r, (c, 256)) for c in range(o, o + n, 256)
                    for g, r in (((mid, 1), (64, 64)), ((mid + 1, 4), (0, 128)))]
        for i in range(0, len(part), 8):
            slot = (NP - 1, G + (o + n) // 256 - 1 + i // 8, "after")
            plan[slot] = plan.get(slot, []) + part[i:i + 8]
    assert sum(g[1] * r[1] * c[1] for cs in plan.values() for g, r, c in cs) == 9 * NP * 128 * S
    return plan


def _kernel(x_hbm, w_hbm, b_hbm, o_hbm, xbuf, obuf, wbuf, bbuf, wa_ref, bias_ref,
            isem, fsem, wsem, osem):
    NB, D, S = x_hbm.shape
    NP = NB // 2
    first = [(0, o, n) for o, n in _split(_IN_FIRST)] + [(1, 0, S)]
    plan = _write_plan(NB, S)

    def x_first(j):
        u, o, n = first[j]
        return pltpu.make_async_copy(
            x_hbm.at[u, :, pl.ds(o, n)], xbuf.at[u, :, pl.ds(o, n)], fsem.at[j])

    def ring(p):
        return p if isinstance(p, int) else jnp.where(p >= _RING, p - _RING, p)

    def x_pair(p):
        return pltpu.make_async_copy(
            x_hbm.at[pl.ds(2 * p, 2)], xbuf.at[pl.ds(2 * ring(p), 2)], isem.at[ring(p)])

    def write(copies):
        for box in copies:
            at = tuple(pl.ds(o, n) for o, n in box)
            pltpu.make_async_copy(obuf.at[at], o_hbm.at[at], osem).start()

    wrows = [(o, min(128, D - o)) for o in range(0, D, 128)]
    wcp = [pltpu.make_async_copy(w_hbm.at[pl.ds(o, n)], wbuf.at[pl.ds(o, n)], wsem.at[m])
           for m, (o, n) in enumerate(wrows)]
    bcp = pltpu.make_async_copy(b_hbm, bbuf, wsem.at[len(wrows)])
    bcp.start()
    for cp in wcp:
        cp.start()
    for j in range(len(first)):
        x_first(j).start(priority=1)
    for p in range(1, _RING):
        x_pair(p).start(priority=1)

    def prepare():
        bcp.wait()
        bias_ref[...] = jnp.broadcast_to(bbuf[...].reshape(1, D).astype(jnp.float32), (128, D)).T

        def tile(m):
            wcp[m].wait()
            wp = _prune(wbuf[pl.ds(*wrows[m]), :])
            wbuf[pl.ds(*wrows[m]), :] = wp
            return jnp.concatenate([wp] * (128 // wp.shape[0]), axis=0).T

        _prepare_weights(tile, wa_ref)

    def put(p, r0, cols, v, first_part_done=lambda: None):
        v = v.astype(obuf.dtype)
        cuts = [r0, *range(r0 // 128 * 128 + 128, r0 + v.shape[0], 128), r0 + v.shape[0]]
        for lo, hi in zip(cuts[:-1], cuts[1:]):
            obuf[9 * p + lo // 128, pl.ds(lo % 128, hi - lo), cols] = v[lo - r0:hi - r0]
            if lo == r0:
                first_part_done()

    def body(t, carry):
        x4, top = carry
        pl.when(t == 0)(prepare)

        @pl.when(t > 0)
        def _():
            x_pair(t).wait()

        @pl.when((t > 0) & (t - 1 + _RING < NP))
        def _():
            x_pair(t - 1 + _RING).start(priority=1)

        for u in range(2):
            slot = 2 * ring(t) + u
            for g0 in range(0, S, 256):
                for j, (uu, o, n) in enumerate(first):
                    if (uu, o) == (u, g0):
                        pl.when(t == 0)(lambda: x_first(j).wait())

                def load(k, j):
                    return xbuf[slot, pl.ds(64 * k, 64), pl.ds(g0 + 128 * j, 128)]

                def start_writes(point):
                    for tt in range(NP):
                        copies = plan.get((tt, (u * S + g0) // 256, point))
                        if copies:
                            pl.when(t == tt)(lambda: write(copies))

                peaks = []

                def store(i, j, v):
                    peaks.append(_fold(jnp.maximum, jnp.abs(v)))
                    put(t, u * D + i * _FH, pl.ds(g0 + 128 * j, 128), v,
                        lambda: (i, j) == (1, 0) and start_writes("late"))

                x4 = jnp.maximum(x4, _super_tile(load, store, wa_ref, bias_ref, start_writes))
                top = functools.reduce(jnp.maximum, peaks, top)
        return x4, top

    x4, top = lax.fori_loop(
        0, NP, body, (jnp.zeros((1, 128), jnp.float32), jnp.zeros((8, 128), jnp.float32)))

    def norm4(sums):
        return jnp.sqrt(jnp.sqrt(jnp.max(sums, axis=1, keepdims=True) + D * 2.0 ** -126))

    w4 = 0.0
    for r in range(0, D, 16):
        w4 += _quartic(wbuf[pl.ds(r, 16), :])
    w4 = jnp.sum(w4, axis=0, keepdims=True)
    top = jnp.max(jnp.max(top, axis=0, keepdims=True), axis=1, keepdims=True)
    safe = (norm4(w4) * norm4(x4) < _SAFE * top) & (top < jnp.inf)
    safe = jnp.max(jnp.where(safe, 1.0, 0.0)) > 0.5

    def wait_writes():
        pltpu.make_async_copy(obuf, obuf, osem).wait()

    pl.when(safe)(wait_writes)

    @pl.when(jnp.logical_not(safe))
    def _():
        wait_writes()
        wt = wbuf[...].T
        bias = bias_ref[...]

        @pl.loop(0, NP)
        def _(p):
            x_pair(p).start()
            x_pair(p).wait()

            @pl.loop(0, S // 128)
            def _(c):
                cols = pl.ds(pl.multiple_of(c * 128, 128), 128)
                for u in range(2):
                    v = jnp.dot(wt, xbuf[2 * ring(p) + u, :, cols],
                                preferred_element_type=jnp.float32)
                    put(p, u * D, cols, v + bias)

        pltpu.make_async_copy(obuf, o_hbm, osem).start()
        wait_writes()


@jax.jit
def pallas_standalone__structured_sparse_n_m__ragged_kernel(
    x: jax.Array,
    w: jax.Array,
    b: jax.Array,
):
    B, S, D = x.shape
    out = pl.pallas_call(
        _kernel,
        in_specs=[pl.BlockSpec(memory_space=pl.ANY)] * 3,
        out_specs=pl.BlockSpec(memory_space=pl.ANY),
        out_shape=jax.ShapeDtypeStruct((B * D // 128, 128, S), x.dtype),
        scratch_shapes=[
            pltpu.VMEM((2 * _RING, D, S), x.dtype),
            pltpu.VMEM((B * D // 128, 128, S), x.dtype),
            pltpu.VMEM((D, D), w.dtype),
            pltpu.VMEM((D,), b.dtype),
            pltpu.VMEM((len(_PASSES), _FH, 128), jnp.bfloat16),
            pltpu.VMEM((D, 128), jnp.float32),
            pltpu.SemaphoreType.DMA((_RING,)),
            pltpu.SemaphoreType.DMA((len(_IN_FIRST) + 1,)),
            pltpu.SemaphoreType.DMA((6,)),
            pltpu.SemaphoreType.DMA(()),
        ],
        compiler_params=pltpu.CompilerParams(
            vmem_limit_bytes=124 * 1024 * 1024,
            disable_bounds_checks=True,
            disable_semaphore_checks=True,
            flags={"XLA_TPU_RESCHEDULE_DMA_DONES": True},
        ),
    )(jnp.transpose(x, (0, 2, 1)), w, b)
    return jnp.transpose(out.reshape(B, D, S), (0, 2, 1))
```

```python
import functools

import jax
import jax.numpy as jnp
from jax import lax
import jax.experimental.pallas as pl
import jax.experimental.pallas.tpu as pltpu

_FH = 288
_RING = 5
_IN_FIRST = (256, 256, 512, 1024, 2048)
_OUT_LAST = (2048, 1024, 512, 256, 256)
_SAFE = 0.75
_PASSES = ("H01", "H02", "H11", "H12", "G01", "G02", "G0h", "O10",
           "I0", "I1", "O00", "O01", "G11", "G12", "G1h", "O11")


def _prune_packed(u):
    mate = lax.broadcasted_iota(jnp.int32, u.shape, 0) ^ 1
    lo = pltpu.bitcast((u << 16) & 0x7FFFFFFF, jnp.float32)
    hi = pltpu.bitcast(u & 0x7FFF0000, jnp.float32)
    big, small = jnp.maximum(lo, hi), jnp.minimum(lo, hi)
    nbig = jnp.take_along_axis(big, mate, axis=0, mode="promise_in_bounds")
    nsmall = jnp.take_along_axis(small, mate, axis=0, mode="promise_in_bounds")
    thr = jnp.maximum(jnp.minimum(big, nbig), jnp.maximum(small, nsmall))
    return u & (jnp.where(lo < thr, 0, 0xFFFF) | jnp.where(hi < thr, 0, -65536))


def _prune(w):
    u = pltpu.bitcast(w, jnp.int32)
    parts = [_prune_packed(u[i:i + 8]) for i in range(0, u.shape[0], 8)]
    return pltpu.bitcast(jnp.concatenate(parts, axis=0), jnp.bfloat16)


def _prepare_weights(tile, wa_ref):
    low = lax.broadcasted_iota(jnp.int32, (_FH, 128), 1) < 64

    def rows(m):
        t = tile(m).astype(jnp.float32)
        return t[:_FH], t[_FH:]

    def put(name, lo, hi=None):
        v = lo if hi is None else jnp.where(low, lo, hi)
        wa_ref[_PASSES.index(name)] = v.astype(wa_ref.dtype)

    a0, b0 = rows(0)
    b0 = b0 * jnp.where(low, 1.0, 0.5)
    put("O10", b0 - a0)
    a1, b1 = rows(1)
    b1 = b1 * jnp.where(low, 1.0, 0.5)
    put("I0", a0 + b1)
    put("O01", a1 - b1)
    ha, hb = a0 + a1, b0 + b1
    a2, b2 = rows(2)
    a2 = a2 * jnp.where(low, 0.5, 1.0)
    put("O11", b2 - a2)
    put("G11", b1, a2)
    a3, b3 = rows(3)
    a3 = a3 * jnp.where(low, 0.5, 1.0)
    put("I1", a2 + b3)
    put("O00", a3 - b3)
    put("G01", a0, b3)
    ha2, hb2 = a2 + a3, b2 + b3
    put("H01", ha, ha2)
    put("H02", ha2, ha)
    put("H11", hb, hb2)
    put("H12", hb2, hb)
    a4, b4 = rows(4)
    tail = a4 * jnp.where(low, -1 / 3, 2 / 3) + b4 * jnp.where(low, 2 / 3, -1 / 3)
    put("G02", tail, a0)
    put("G12", tail, b1)
    put("G0h", b3, tail)
    put("G1h", a2, tail)


def _fold(op, v):
    return functools.reduce(op, [v[i:i + 8] for i in range(0, v.shape[0], 8)])


def _quartic(v):
    v = v.astype(jnp.float32)
    v = v * v
    return _fold(jnp.add, v * v)


def _super_tile(x, store, wa_ref, bias_ref, start_writes):
    quartic = {}

    def wide(k, j):
        v = x(k, j).astype(jnp.float32)
        if (k, j) not in quartic:
            quartic[k, j] = _quartic(v)
        return v

    def diff(p, q, cp=1.0, cq=1.0):
        p, q = wide(*p), wide(*q)
        return (p if cp == 1 else p * cp) - (q if cq == 1 else q * cq)

    def mm(name, lo, hi):
        rhs = jnp.concatenate([lo, hi], axis=0).astype(jnp.bfloat16)
        return jnp.dot(wa_ref[_PASSES.index(name)], rhs, preferred_element_type=jnp.float32)

    start_writes("before")
    h01 = mm("H01", x(2, 0), x(7, 1))
    h02 = mm("H02", x(6, 1), x(3, 0))
    h11 = mm("H11", x(0, 1), x(5, 0))
    h12 = mm("H12", x(4, 0), x(1, 1))
    c00 = h01 + bias_ref[pl.ds(0, _FH)] + h02
    c01 = c00 + h02
    c10 = h11 + bias_ref[pl.ds(_FH, _FH)] + h12
    c11 = c10 + h12

    g1 = mm("G01", diff((0, 0), (2, 0)), diff((7, 0), (5, 0)))
    g2 = mm("G02", wide(8, 0), diff((1, 0), (3, 0)))
    gh = mm("G0h", diff((6, 0), (4, 0)), wide(8, 0))
    o10 = mm("O10", diff((0, 0), (0, 1)), diff((1, 0), (1, 1), cp=2.0))
    s = g1 + g2 + gh
    c00 = c00 + (s + gh)
    c10 = c10 + (s + g2) + o10

    i0 = mm("I0", diff((0, 1), (2, 0)), diff((1, 1), (3, 0), cq=2.0))
    i1 = mm("I1", diff((4, 0), (6, 1), cp=2.0), diff((5, 0), (7, 1)))
    o00 = mm("O00", diff((6, 0), (6, 1), cp=2.0), diff((7, 0), (7, 1)))
    o01 = mm("O01", diff((2, 1), (2, 0)), diff((3, 1), (3, 0), cq=2.0))
    store(1, 0, c10 - i0)
    store(0, 0, c00 + i1 + o00)
    c01 = c01 + i0 + o01
    c11 = c11 - i1

    g1 = mm("G11", diff((2, 1), (0, 1)), diff((5, 1), (7, 1)))
    g2 = mm("G12", wide(8, 1), diff((3, 1), (1, 1)))
    gh = mm("G1h", diff((4, 1), (6, 1)), wide(8, 1))
    o11 = mm("O11", diff((4, 1), (4, 0), cq=2.0), diff((5, 1), (5, 0)))
    s = g1 + g2 + gh
    store(0, 1, c01 + gh + s)
    store(1, 1, c11 + g2 + s + o11)
    start_writes("after")
    return jnp.maximum(*(
        jnp.sum(functools.reduce(jnp.add, [quartic[k, j] for k in range(9)]), axis=0, keepdims=True)
        for j in range(2)))


def _split(sizes):
    return [(sum(sizes[:j]), sizes[j]) for j in range(len(sizes))]


def _write_plan(NB, S):
    NP, G = NB // 2, S // 256

    def strided(groups):
        return [(groups(r), (r, 8), (c, 1024)) for r in range(0, 128, 8) for c in range(0, S, 1024)]

    def pair(p):
        return strided(lambda r: (9 * p, 9))

    bulk = [c for p in range(NP - 2) for c in pair(p)]
    plan = {(NP // 2 - 1, 2 * G - 1, "late"): bulk[:16], (NP // 2, 0, "before"): bulk[16:68]}
    done = 68
    for i in range((NP // 2 - 1) * G):
        t = NP // 2 + i // G
        end = min(76 + 8 * i, 64 * t)
        plan[t, G + i % G, "before"], done = bulk[done:end], end
    plan[NP - 1, 0, "before"] = pair(NP - 2)

    mid = 9 * (NP - 1) + 4
    part = strided(lambda r: (mid - 4, 5 if r < 64 else 4))
    for i in range(len(part) // 16):
        plan[NP - 1, G + 2 * i, "before"] = part[16 * i:16 * i + 16]
    for o, n in _split(_OUT_LAST):
        if n >= 1024:
            part = [(g, (r + h, 8), (c, 1024))
                    for r in range(0, 64, 8) for c in range(o, o + n, 1024)
                    for g, h in (((mid + 1, 4), 0), ((mid, 5), 64))]
        else:
            part = [(g, r, (c, 256)) for c in range(o, o + n, 256)
                    for g, r in (((mid, 1), (64, 64)), ((mid + 1, 4), (0, 128)))]
        for i in range(0, len(part), 8):
            slot = (NP - 1, G + (o + n) // 256 - 1 + i // 8, "after")
            plan[slot] = plan.get(slot, []) + part[i:i + 8]
    assert sum(g[1] * r[1] * c[1] for cs in plan.values() for g, r, c in cs) == 9 * NP * 128 * S
    return plan


def _kernel(x_hbm, w_hbm, b_hbm, o_hbm, xbuf, obuf, wbuf, bbuf, wa_ref, bias_ref,
            isem, fsem, wsem, osem):
    NB, D, S = x_hbm.shape
    NP = NB // 2
    first = [(0, o, n) for o, n in _split(_IN_FIRST)] + [(1, 0, S)]
    plan = _write_plan(NB, S)

    def x_first(j):
        u, o, n = first[j]
        return pltpu.make_async_copy(
            x_hbm.at[u, :, pl.ds(o, n)], xbuf.at[u, :, pl.ds(o, n)], fsem.at[j])

    def ring(p):
        return p if isinstance(p, int) else jnp.where(p >= _RING, p - _RING, p)

    def x_pair(p):
        return pltpu.make_async_copy(
            x_hbm.at[pl.ds(2 * p, 2)], xbuf.at[pl.ds(2 * ring(p), 2)], isem.at[ring(p)])

    def write(copies):
        for box in copies:
            at = tuple(pl.ds(o, n) for o, n in box)
            pltpu.make_async_copy(obuf.at[at], o_hbm.at[at], osem).start()

    wrows = [(o, min(128, D - o)) for o in range(0, D, 128)]
    wcp = [pltpu.make_async_copy(w_hbm.at[pl.ds(o, n)], wbuf.at[pl.ds(o, n)], wsem.at[m])
           for m, (o, n) in enumerate(wrows)]
    bcp = pltpu.make_async_copy(b_hbm, bbuf, wsem.at[len(wrows)])
    bcp.start()
    for cp in wcp:
        cp.start()
    for j in range(len(first)):
        x_first(j).start(priority=1)
    for p in range(1, _RING):
        x_pair(p).start(priority=1)

    def prepare():
        bcp.wait()
        bias_ref[...] = jnp.broadcast_to(bbuf[...].reshape(1, D).astype(jnp.float32), (128, D)).T

        def tile(m):
            wcp[m].wait()
            wp = _prune(wbuf[pl.ds(*wrows[m]), :])
            wbuf[pl.ds(*wrows[m]), :] = wp
            return jnp.concatenate([wp] * (128 // wp.shape[0]), axis=0).T

        _prepare_weights(tile, wa_ref)

    def put(p, r0, cols, v, first_part_done=None):
        v = v.astype(obuf.dtype)
        cuts = [r0, *range(r0 // 128 * 128 + 128, r0 + v.shape[0], 128), r0 + v.shape[0]]
        for lo, hi in zip(cuts[:-1], cuts[1:]):
            obuf[9 * p + lo // 128, pl.ds(lo % 128, hi - lo), cols] = v[lo - r0:hi - r0]
            if lo == r0 and first_part_done:
                first_part_done()

    def body(t, carry):
        x4, top = carry
        pl.when(t == 0)(prepare)

        @pl.when(t > 0)
        def _():
            x_pair(t).wait()

        @pl.when((t > 0) & (t - 1 + _RING < NP))
        def _():
            x_pair(t - 1 + _RING).start(priority=1)

        for u in range(2):
            slot = 2 * ring(t) + u
            for g0 in range(0, S, 256):
                for j, (uu, o, n) in enumerate(first):
                    if (uu, o) == (u, g0):
                        pl.when(t == 0)(lambda: x_first(j).wait())

                def load(k, j):
                    return xbuf[slot, pl.ds(64 * k, 64), pl.ds(g0 + 128 * j, 128)]

                def start_writes(point):
                    for tt in range(NP):
                        copies = plan.get((tt, (u * S + g0) // 256, point))
                        if copies:
                            pl.when(t == tt)(lambda: write(copies))

                peaks = []

                def store(i, j, v):
                    peaks.append(_fold(jnp.maximum, jnp.abs(v)))
                    late = functools.partial(start_writes, "late") if (i, j) == (1, 0) else None
                    put(t, u * D + i * _FH, pl.ds(g0 + 128 * j, 128), v, late)

                x4 = jnp.maximum(x4, _super_tile(load, store, wa_ref, bias_ref, start_writes))
                top = functools.reduce(jnp.maximum, peaks, top)
        return x4, top

    x4, top = lax.fori_loop(
        0, NP, body, (jnp.zeros((1, 128), jnp.float32), jnp.zeros((8, 128), jnp.float32)))

    def norm4(sums):
        return jnp.sqrt(jnp.sqrt(jnp.max(sums, axis=1, keepdims=True) + D * 2.0 ** -126))

    w4 = 0.0
    for r in range(0, D, 16):
        w4 += _quartic(wbuf[pl.ds(r, 16), :])
    w4 = jnp.sum(w4, axis=0, keepdims=True)
    top = jnp.max(jnp.max(top, axis=0, keepdims=True), axis=1, keepdims=True)
    safe = (norm4(w4) * norm4(x4) < _SAFE * top) & (top < jnp.inf)
    safe = jnp.max(jnp.where(safe, 1.0, 0.0)) > 0.5

    def wait_writes():
        pltpu.make_async_copy(obuf, obuf, osem).wait()

    def recompute():
        wait_writes()
        wt = wbuf[...].T
        bias = bias_ref[...]

        @pl.loop(0, NP)
        def _(p):
            x_pair(p).start()
            x_pair(p).wait()

            @pl.loop(0, S // 128)
            def _(c):
                cols = pl.ds(pl.multiple_of(c * 128, 128), 128)
                for u in range(2):
                    v = jnp.dot(wt, xbuf[2 * ring(p) + u, :, cols],
                                preferred_element_type=jnp.float32)
                    put(p, u * D, cols, v + bias)

        pltpu.make_async_copy(obuf, o_hbm, osem).start()
        wait_writes()

    lax.cond(safe, wait_writes, recompute)


@jax.jit
def pallas_standalone__structured_sparse_n_m__ragged_kernel(
    x: jax.Array,
    w: jax.Array,
    b: jax.Array,
):
    B, S, D = x.shape
    out = pl.pallas_call(
        _kernel,
        in_specs=[pl.BlockSpec(memory_space=pl.ANY)] * 3,
        out_specs=pl.BlockSpec(memory_space=pl.ANY),
        out_shape=jax.ShapeDtypeStruct((B * D // 128, 128, S), x.dtype),
        scratch_shapes=[
            pltpu.VMEM((2 * _RING, D, S), x.dtype),
            pltpu.VMEM((B * D // 128, 128, S), x.dtype),
            pltpu.VMEM((D, D), w.dtype),
            pltpu.VMEM((D,), b.dtype),
            pltpu.VMEM((len(_PASSES), _FH, 128), jnp.bfloat16),
            pltpu.VMEM((D, 128), jnp.float32),
            pltpu.SemaphoreType.DMA((_RING,)),
            pltpu.SemaphoreType.DMA((len(_IN_FIRST) + 1,)),
            pltpu.SemaphoreType.DMA((6,)),
            pltpu.SemaphoreType.DMA(()),
        ],
        compiler_params=pltpu.CompilerParams(
            vmem_limit_bytes=124 * 1024 * 1024,
            disable_bounds_checks=True,
            disable_semaphore_checks=True,
            flags={"XLA_TPU_RESCHEDULE_DMA_DONES": True},
        ),
    )(jnp.transpose(x, (0, 2, 1)), w, b)
    return jnp.transpose(out.reshape(B, D, S), (0, 2, 1))
```
